```python
import os as _os
_os.environ.setdefault("JAX_PLATFORMS", "cpu")
import jax
import jax.numpy as jnp

def _softmax(x, axis=-1):
    return jax.nn.softmax(x, axis=axis)
def _gelu(x):
    return jax.nn.gelu(x, approximate=True)
def _silu(x):
    return jax.nn.silu(x)
def _sigmoid(x):
    return jax.nn.sigmoid(x)
def _layernorm(x, axis=-1, eps=1e-5):
    m = jnp.mean(x, axis=axis, keepdims=True)
    v = jnp.var(x, axis=axis, keepdims=True)
    return (x - m) / jnp.sqrt(v + eps)
def _scatter_add(tgt, idx, src, axis=0):
    return tgt.at[idx].add(src)
def _segment_sum(src, seg, n):
    return jax.ops.segment_sum(src, seg, n)
class _Rng:
    def __init__(self, key):
        self._k = key
    def _next(self):
        self._k, sub = jax.random.split(self._k)
        return sub
    def normal(self, shape):
        return jax.random.normal(self._next(), shape, dtype=jnp.bfloat16)
    def randint(self, lo, hi, shape):
        return jax.random.randint(self._next(), shape, lo, hi, dtype=jnp.int32)
    def uniform(self, shape, lo=0.0, hi=1.0):
        return jax.random.uniform(self._next(), shape, jnp.bfloat16, lo, hi)
    def permutation(self, n):
        return jax.random.permutation(self._next(), n)


kernel_name = 'interleave_layers__linear_kernel_hedgehog__dense_activation_silu__prompt'

def setup_inputs():
    _rng = _Rng(jax.random.key(int.from_bytes(__import__("os").urandom(4), "little")))
    _w = (lambda a: (lambda t: t.astype(jnp.bfloat16) if jnp.issubdtype(t.dtype, jnp.floating) else t)(jnp.asarray(a)))
    def _A_setup():
        B, S, D, H = 1, 2048, 640, 32
        Dh = D // H
        return {
            "x": _w((lambda *s: _rng.normal(s) * 0.05)(B, S, D)),
            "wqkv": _w((lambda *s: _rng.normal(s) * 0.4)(D, 3 * D)),
            "w_phi": _w((lambda *s: _rng.normal(s) * 0.4)(H, Dh, Dh) * (Dh ** -0.5)),
            "wo": _w((lambda *s: _rng.normal(s) * 0.05)(D, D)),
        }
    _A_in = _A_setup()

    def _B_setup():
        B, S, D, F = 1, 2048, 640, 1728
        return {
            "x": _w((lambda *s: _rng.normal(s) * 0.05)(B, S, D)),
            "w1": _w((lambda *s: _rng.normal(s) * 1.6)(D, F) * (D ** -0.5)),
            "w2": _w((lambda *s: _rng.normal(s) * 1.6)(F, D) * (F ** -0.5)),
        }
    _B_in = _B_setup()

    return {
        "A_x": _A_in["x"],
        "A_wqkv": _A_in["wqkv"],
        "A_w_phi": _A_in["w_phi"],
        "A_wo": _A_in["wo"],
        "B_x": _B_in["x"],
        "B_w1": _B_in["w1"],
        "B_w2": _B_in["w2"],
    }

def reference(A_x, A_wqkv, A_w_phi, A_wo, B_x, B_w1, B_w2):
    def _A_ref(x, wqkv, w_phi, wo):
        B, S, D = x.shape
        H = 32; Dh = D // H
        qkv = (lambda x, *d: x.transpose(*d))((x @ wqkv).reshape(B, S, 3, H, Dh), 2, 0, 3, 1, 4)
        q, k, v = qkv[0], qkv[1], qkv[2]
        pq = jnp.einsum("bhsd,hdf->bhsf", q, w_phi)
        pk = jnp.einsum("bhsd,hdf->bhsf", k, w_phi)
        phi_q = jnp.concatenate([_softmax(pq, axis=-1), _softmax(-pq, axis=-1)], axis=-1)
        phi_k = jnp.concatenate([_softmax(pk, axis=-1), _softmax(-pk, axis=-1)], axis=-1)
        kv = jnp.einsum("bhsf,bhsd->bhfd", phi_k, v)
        z  = jnp.einsum("bhsf->bhf", phi_k)
        num = jnp.einsum("bhqf,bhfd->bhqd", phi_q, kv)
        den = jnp.einsum("bhqf,bhf->bhq", phi_q, z)[..., None] + 1e-6
        o = num / den
        return (lambda x, *d: x.transpose(*d))(o, 0, 2, 1, 3).reshape(B, S, D) @ wo

    def _B_ref(x, w1, w2):
        h = jnp.einsum("bsd,df->bsf", x, w1)
        h = _silu(h)
        out = jnp.einsum("bsf,fd->bsd", h, w2)
        return out

    x = A_x
    x = x + _A_ref(_layernorm(x, axis=-1), A_wqkv, A_w_phi, A_wo)
    x = x + _B_ref(_layernorm(x, axis=-1), B_w1, B_w2)
    x = x + _A_ref(_layernorm(x, axis=-1), A_wqkv, A_w_phi, A_wo)
    x = x + _B_ref(_layernorm(x, axis=-1), B_w1, B_w2)
    return x
```

```python
import functools

import jax
import jax.numpy as jnp
from jax import lax
import jax.experimental.pallas as pl
import jax.experimental.pallas.tpu as pltpu

S = 2048
D = 640
H = 32
DH = 20
F = 1728
NG = 4
HG = 8
GROWS = HG * DH
GPHI = 2 * GROWS
VROWS = GROWS + 16

TS = 256
NT = S // TS

LN_EPS = 1e-5
DEN_EPS = 1e-6

_NT_DIMS = (((1,), (1,)), ((), ()))


def _dot(a, b):
    return jnp.dot(a, b, preferred_element_type=jnp.float32)


def _dot_nt(a, b):
    return lax.dot_general(a, b, _NT_DIMS, preferred_element_type=jnp.float32)


def _layernorm(x):
    m = jnp.mean(x, axis=-1, keepdims=True)
    xc = x - m
    v = jnp.mean(xc * xc, axis=-1, keepdims=True)
    return xc * lax.rsqrt(v + LN_EPS)


def _phi_t(p_t):
    ts = p_t.shape[1]
    p = p_t.reshape(NG, DH, HG, ts)
    pmax = jnp.max(p, axis=1, keepdims=True)
    pmin = jnp.min(p, axis=1, keepdims=True)
    ep = jnp.exp(p - pmax)
    en = jnp.exp(pmin - p)
    rp = pl.reciprocal(jnp.sum(ep, axis=1, keepdims=True), approx=False)
    rn = pl.reciprocal(jnp.sum(en, axis=1, keepdims=True), approx=False)
    pos = (ep * rp).astype(jnp.bfloat16)
    neg = (en * rn).astype(jnp.bfloat16)
    phi = jnp.concatenate([pos, neg], axis=1)
    return phi.reshape(2 * D, ts)


def _kernel(x_ref, wqkv_ref, wphi_ref, wo_ref, w1_ref, w2_ref, o_ref,
            xres_ref, phiq_ref, wat_ref, tmpw_ref, acc_ref, kvz_ref):
    phase = pl.program_id(0)
    t = pl.program_id(1)
    col = pl.multiple_of(t * TS, TS)

    @pl.when(jnp.logical_and(phase == 0, t == 0))
    def _prep():
        tmpw_ref[...] = jnp.zeros(tmpw_ref.shape, tmpw_ref.dtype)
        for h in range(H):
            tmpw_ref[pl.ds(DH * h, DH), pl.ds(0, DH)] = (
                wphi_ref[h].astype(jnp.float32))
        wphi2 = tmpw_ref[...].astype(jnp.bfloat16)
        r = lax.broadcasted_iota(jnp.int32, (D, 128), 0)
        k = lax.broadcasted_iota(jnp.int32, (D, 128), 1)
        onehot = (k == (r % GROWS) // HG).astype(jnp.bfloat16)
        mfull = _dot_nt(onehot, wphi2)
        r = lax.broadcasted_iota(jnp.int32, (D, D), 0)
        c = lax.broadcasted_iota(jnp.int32, (D, D), 1)
        head_r = (r // GROWS) * HG + r % HG
        mt = jnp.where(c // DH == head_r, mfull, 0.0).astype(jnp.bfloat16)
        wat_ref[pl.ds(0, D), :] = _dot_nt(mt, wqkv_ref[:, pl.ds(0, D)]).astype(jnp.bfloat16)
        wat_ref[pl.ds(D, D), :] = _dot_nt(mt, wqkv_ref[:, pl.ds(D, D)]).astype(jnp.bfloat16)
        eye = (r == c).astype(jnp.bfloat16)
        wat_ref[pl.ds(2 * D, D), :] = _dot_nt(eye, wqkv_ref[:, pl.ds(2 * D, D)]).astype(jnp.bfloat16)
        acc_ref[...] = jnp.zeros(acc_ref.shape, acc_ref.dtype)

    @pl.when(jnp.logical_and(phase >= 1, t == 0))
    def _finalize():
        r = lax.broadcasted_iota(jnp.int32, (VROWS, GPHI), 0)
        c = lax.broadcasted_iota(jnp.int32, (VROWS, GPHI), 1)
        head_r = jnp.where(r < GROWS, r // DH, r - GROWS)
        keep = head_r == c % HG
        for g in range(NG):
            kvz_ref[g] = jnp.where(keep, acc_ref[g], 0.0).astype(jnp.bfloat16)
        acc_ref[...] = jnp.zeros(acc_ref.shape, acc_ref.dtype)

    @pl.when(phase >= 1)
    def _back():
        x_t = xres_ref[pl.ds(col, TS), :]
        o_parts = []
        for g in range(NG):
            pg = phiq_ref[pl.ds(GPHI * g, GPHI), pl.ds(col, TS)]
            den = _dot(kvz_ref[g, pl.ds(GROWS, 16), :], pg)
            rden = pl.reciprocal(den[:HG] + DEN_EPS, approx=False)
            pgn = (pg.astype(jnp.float32).reshape(2 * DH, HG, TS) * rden[None]
                   ).reshape(GPHI, TS).astype(jnp.bfloat16)
            o_parts.append(_dot(kvz_ref[g, pl.ds(0, GROWS), :], pgn))
        o_t = jnp.concatenate(o_parts, axis=0)
        o = o_t.T.astype(jnp.bfloat16)
        x1 = x_t + _dot(o, wo_ref[...])
        xn = _layernorm(x1).astype(jnp.bfloat16)
        hdn = _dot(xn, w1_ref[...])
        hdn = (hdn * jax.nn.sigmoid(hdn)).astype(jnp.bfloat16)
        x2 = x1 + _dot(hdn, w2_ref[...])
        xres_ref[pl.ds(col, TS), :] = x2

        @pl.when(phase == 2)
        def _():
            o_ref[...] = x2.astype(o_ref.dtype)

    @pl.when(phase <= 1)
    def _front():
        @pl.when(phase == 0)
        def _():
            xres_ref[pl.ds(col, TS), :] = x_ref[...].astype(jnp.float32)

        x_t = xres_ref[pl.ds(col, TS), :]
        xn = _layernorm(x_t).astype(jnp.bfloat16)
        y_t = _dot_nt(wat_ref[...], xn)
        phiq_ref[:, pl.ds(col, TS)] = _phi_t(y_t[:D])
        phik = _phi_t(y_t[D:2 * D])
        v_t = y_t[2 * D:].astype(jnp.bfloat16)
        ones = jnp.ones((VROWS - GROWS, TS), jnp.bfloat16)
        for g in range(NG):
            vaug = jnp.concatenate([v_t[GROWS * g:GROWS * (g + 1)], ones], axis=0)
            acc_ref[g] += _dot_nt(vaug, phik[GPHI * g:GPHI * (g + 1)])


@jax.jit
def pallas_interleave_layers__linear_kernel_hedgehog__dense_activation_silu__prompt_kernel(
    A_x: jax.Array,
    A_wqkv: jax.Array,
    A_w_phi: jax.Array,
    A_wo: jax.Array,
    B_x: jax.Array,
    B_w1: jax.Array,
    B_w2: jax.Array,
):
    del B_x
    whole = lambda shape: pl.BlockSpec(shape, lambda p, t: (0,) * len(shape))
    return pl.pallas_call(
        _kernel,
        grid=(3, NT),
        in_specs=[
            pl.BlockSpec((None, TS, D),
                         lambda p, t: (0, jnp.where(p == 0, t, NT - 1), 0)),
            whole((D, 3 * D)),
            whole((H, DH, DH)),
            whole((D, D)),
            whole((D, F)),
            whole((F, D)),
        ],
        out_specs=pl.BlockSpec((None, TS, D),
                               lambda p, t: (0, jnp.where(p == 2, t, 0), 0)),
        out_shape=jax.ShapeDtypeStruct((1, S, D), jnp.bfloat16),
        scratch_shapes=[
            pltpu.VMEM((S, D), jnp.float32),
            pltpu.VMEM((2 * D, S), jnp.bfloat16),
            pltpu.VMEM((3 * D, D), jnp.bfloat16),
            pltpu.VMEM((D, 128), jnp.float32),
            pltpu.VMEM((NG, VROWS, GPHI), jnp.float32),
            pltpu.VMEM((NG, VROWS, GPHI), jnp.bfloat16),
        ],
        compiler_params=pltpu.CompilerParams(
            dimension_semantics=("arbitrary", "arbitrary"),
            vmem_limit_bytes=100 * 1024 * 1024,
        ),
    )(A_x, A_wqkv, A_w_phi, A_wo, B_w1, B_w2)
```

```python
import jax
import jax.numpy as jnp
from jax import lax
import jax.experimental.pallas as pl
import jax.experimental.pallas.tpu as pltpu

S = 2048
D = 640
H = 32
DH = 20
F = 1728
HG = 2
NG = H // HG
GROWS = HG * DH
GPHI = 2 * GROWS
VROWS = 64

TS = 512
NT = S // TS

LN_EPS = 1e-5
DEN_EPS = 1e-6

_NT_DIMS = (((1,), (1,)), ((), ()))


def _dot(a, b):
    return jnp.dot(a, b, preferred_element_type=jnp.float32)


def _dot_nt(a, b):
    return lax.dot_general(a, b, _NT_DIMS, preferred_element_type=jnp.float32)


def _layernorm(x):
    m = jnp.mean(x, axis=-1, keepdims=True)
    xc = x - m
    v = jnp.mean(xc * xc, axis=-1, keepdims=True)
    return xc * lax.rsqrt(v + LN_EPS)


def _phi_t(p_t):
    ts = p_t.shape[1]
    p = p_t.reshape(NG, 5, 8, ts)

    def allred(x, op):
        x = op(x, pltpu.roll(x, 2, 1))
        x = op(x, pltpu.roll(x, 4, 1))
        return x[:, None]

    pmax = allred(jnp.max(p, axis=1), jnp.maximum)
    pmin = allred(jnp.min(p, axis=1), jnp.minimum)
    ep = jnp.exp(p - pmax)
    en = jnp.exp(pmin - p)
    rp = pl.reciprocal(allred(jnp.sum(ep, axis=1), jnp.add), approx=False)
    rn = pl.reciprocal(allred(jnp.sum(en, axis=1), jnp.add), approx=False)
    phi = jnp.concatenate([ep * rp, en * rn], axis=1)
    return phi.reshape(2 * D, ts).astype(jnp.bfloat16)


def _kernel(x_ref, wqkv_hbm, wphi_hbm, wo_hbm, w1t_hbm, w2_hbm, o_ref,
            xres_ref, phiq_ref, wat_ref, tmpw_ref, acc_ref, kvz_ref,
            wqkv_ref, wphi_ref, wo_ref, w1t_ref, w2_ref, sems):
    phase = pl.program_id(0)
    t = pl.program_id(1)
    col = pl.multiple_of(t * TS, TS)

    copies = [
        pltpu.make_async_copy(src, dst, sems.at[i])
        for i, (src, dst) in enumerate([
            (wphi_hbm, wphi_ref), (wqkv_hbm, wqkv_ref), (wo_hbm, wo_ref),
            (w1t_hbm, w1t_ref), (w2_hbm, w2_ref)])
    ]

    @pl.when(jnp.logical_and(phase == 0, t == 0))
    def _prep():
        for c in copies:
            c.start()
        copies[0].wait()
        copies[1].wait()
        tmpw_ref[...] = jnp.zeros(tmpw_ref.shape, tmpw_ref.dtype)
        for h in range(H):
            tmpw_ref[pl.ds(DH * h, DH), pl.ds(0, DH)] = (
                wphi_ref[h].astype(jnp.float32))
        wphi2 = tmpw_ref[...].astype(jnp.bfloat16)
        RB = 160
        for b in range(D // RB):
            lo = min(128 * b, D - 256)
            r = RB * b + lax.broadcasted_iota(jnp.int32, (RB, 128), 0)
            k = lax.broadcasted_iota(jnp.int32, (RB, 128), 1)
            onehot = (k == (r % GROWS) // HG).astype(jnp.bfloat16)
            mfull = _dot_nt(onehot, wphi2[lo:lo + 256])
            r = RB * b + lax.broadcasted_iota(jnp.int32, (RB, 256), 0)
            c = lo + lax.broadcasted_iota(jnp.int32, (RB, 256), 1)
            head_r = (r // GROWS) * HG + r % HG
            mt = jnp.where(c // DH == head_r, mfull, 0.0).astype(jnp.bfloat16)
            for part in range(2):
                wat_ref[pl.ds(part * D + RB * b, RB), :] = _dot_nt(
                    mt, wqkv_ref[:, pl.ds(part * D + lo, 256)]).astype(jnp.bfloat16)
        r = lax.broadcasted_iota(jnp.int32, (128, 128), 0)
        c = lax.broadcasted_iota(jnp.int32, (128, 128), 1)
        eye = (r == c).astype(jnp.bfloat16)
        for b in range(D // 128):
            wat_ref[pl.ds(2 * D + 128 * b, 128), :] = _dot_nt(
                eye, wqkv_ref[:, pl.ds(2 * D + 128 * b, 128)]).astype(jnp.bfloat16)
        acc_ref[...] = jnp.zeros(acc_ref.shape, acc_ref.dtype)

    @pl.when(jnp.logical_and(phase >= 1, t == 0))
    def _finalize():
        @pl.when(phase == 1)
        def _():
            for c in copies[2:]:
                c.wait()

        r = lax.broadcasted_iota(jnp.int32, (VROWS, GPHI), 0)
        c = lax.broadcasted_iota(jnp.int32, (VROWS, GPHI), 1)
        head_r = jnp.where(r < GROWS, r // DH,
                           jnp.where(r < 48, 0, jnp.where(r < 56, 1, (r - 56) // 4)))
        keep = head_r == c % HG
        for g in range(NG):
            kvz_ref[g] = jnp.where(keep, acc_ref[g], 0.0).astype(jnp.bfloat16)
        acc_ref[...] = jnp.zeros(acc_ref.shape, acc_ref.dtype)

    @pl.when(phase >= 1)
    def _back():
        x_t = xres_ref[pl.ds(col, TS), :]
        o_parts = []
        for g in range(NG):
            pg = phiq_ref[pl.ds(GPHI * g, GPHI), pl.ds(col, TS)]
            res = _dot(kvz_ref[g], pg)
            ra = pl.reciprocal(res[40:48] + DEN_EPS, approx=False)
            rb = pl.reciprocal(res[48:56] + DEN_EPS, approx=False)
            rm = pl.reciprocal(res[56:64] + DEN_EPS, approx=False)
            o_parts += [res[0:8] * ra, res[8:16] * ra, res[16:24] * rm,
                        res[24:32] * rb, res[32:40] * rb]
        o_t = jnp.concatenate(o_parts, axis=0)
        o = o_t.T.astype(jnp.bfloat16)
        x1 = x_t + _dot(o, wo_ref[...])
        xn = _layernorm(x1).astype(jnp.bfloat16)
        hdn = _dot_nt(xn, w1t_ref[...])
        hdn = (hdn * jax.nn.sigmoid(hdn)).astype(jnp.bfloat16)
        x2 = x1 + _dot(hdn, w2_ref[...])
        xres_ref[pl.ds(col, TS), :] = x2

        @pl.when(phase == 2)
        def _():
            o_ref[...] = x2.astype(o_ref.dtype)

    @pl.when(phase <= 1)
    def _front():
        @pl.when(phase == 0)
        def _():
            xres_ref[pl.ds(col, TS), :] = x_ref[...].astype(jnp.float32)

        x_t = xres_ref[pl.ds(col, TS), :]
        xn = _layernorm(x_t).astype(jnp.bfloat16)
        y_t = _dot_nt(wat_ref[...], xn)
        phiq_ref[:, pl.ds(col, TS)] = _phi_t(y_t[:D])
        phik = _phi_t(y_t[D:2 * D])
        v_t = y_t[2 * D:]
        ones = jnp.ones((VROWS - GROWS, TS), jnp.float32)
        for g in range(NG):
            vaug = jnp.concatenate([v_t[GROWS * g:GROWS * (g + 1)], ones],
                                   axis=0).astype(jnp.bfloat16)
            acc_ref[g] += _dot_nt(vaug, phik[GPHI * g:GPHI * (g + 1)])


@jax.jit
def pallas_interleave_layers__linear_kernel_hedgehog__dense_activation_silu__prompt_kernel(
    A_x: jax.Array,
    A_wqkv: jax.Array,
    A_w_phi: jax.Array,
    A_wo: jax.Array,
    B_x: jax.Array,
    B_w1: jax.Array,
    B_w2: jax.Array,
):
    del B_x
    hbm = pl.BlockSpec(memory_space=pl.ANY)
    return pl.pallas_call(
        _kernel,
        grid=(3, NT),
        in_specs=[
            pl.BlockSpec((None, TS, D),
                         lambda p, t: (0, jnp.where(p == 0, t, NT - 1), 0)),
            hbm, hbm, hbm, hbm, hbm,
        ],
        out_specs=pl.BlockSpec((None, TS, D),
                               lambda p, t: (0, jnp.where(p == 2, t, 0), 0)),
        out_shape=jax.ShapeDtypeStruct((1, S, D), jnp.bfloat16),
        scratch_shapes=[
            pltpu.VMEM((S, D), jnp.float32),
            pltpu.VMEM((2 * D, S), jnp.bfloat16),
            pltpu.VMEM((3 * D, D), jnp.bfloat16),
            pltpu.VMEM((D, 128), jnp.float32),
            pltpu.VMEM((NG, VROWS, GPHI), jnp.float32),
            pltpu.VMEM((NG, VROWS, GPHI), jnp.bfloat16),
            pltpu.VMEM((D, 3 * D), jnp.bfloat16),
            pltpu.VMEM((H, DH, DH), jnp.bfloat16),
            pltpu.VMEM((D, D), jnp.bfloat16),
            pltpu.VMEM((F, D), jnp.bfloat16),
            pltpu.VMEM((F, D), jnp.bfloat16),
            pltpu.SemaphoreType.DMA((5,)),
        ],
        compiler_params=pltpu.CompilerParams(
            dimension_semantics=("arbitrary", "arbitrary"),
            vmem_limit_bytes=100 * 1024 * 1024,
        ),
    )(A_x, A_wqkv, A_w_phi, A_wo, B_w1.T, B_w2)
```

```python
import jax
import jax.numpy as jnp
from jax import lax
import jax.experimental.pallas as pl
import jax.experimental.pallas.tpu as pltpu

S = 2048
D = 640
H = 32
DH = 20
F = 1728
HG = 2
NG = H // HG
GROWS = HG * DH
GPHI = 2 * GROWS
VROWS = 64

SUB = 128
NSUBS = (8, 2, 4)

LN_EPS = 1e-5
DEN_EPS = 1e-6

_NT_DIMS = (((1,), (1,)), ((), ()))


def _dot(a, b):
    return jnp.dot(a, b, preferred_element_type=jnp.float32)


def _dot_nt(a, b):
    return lax.dot_general(a, b, _NT_DIMS, preferred_element_type=jnp.float32)


def _layernorm(x):
    m = jnp.mean(x, axis=-1, keepdims=True)
    xc = x - m
    v = jnp.mean(xc * xc, axis=-1, keepdims=True)
    return xc * lax.rsqrt(v + LN_EPS)


def _phi_t(p_t):
    ts = p_t.shape[1]
    p = p_t.reshape(NG, 5, 8, ts)

    def allred(x, op):
        x = op(x, pltpu.roll(x, 2, 1))
        x = op(x, pltpu.roll(x, 4, 1))
        return x[:, None]

    pmax = allred(jnp.max(p, axis=1), jnp.maximum)
    pmin = allred(jnp.min(p, axis=1), jnp.minimum)
    ep = jnp.exp(p - pmax)
    en = jnp.exp(pmin - p)
    rp = pl.reciprocal(allred(jnp.sum(ep, axis=1), jnp.add), approx=False)
    rn = pl.reciprocal(allred(jnp.sum(en, axis=1), jnp.add), approx=False)
    phi = jnp.concatenate([ep * rp, en * rn], axis=1)
    return phi.reshape(2 * D, ts).astype(jnp.bfloat16)


def _kernel(x_hbm, wqkv_hbm, wphi_hbm, wo_hbm, w1t_hbm, w2_hbm, o_hbm,
            xio_ref, xres_ref, phiq_ref, wat_ref, tmpw_ref, acc_ref, kvz_ref,
            wqkv_ref, wphi_ref, wo_ref, w1t_ref, w2_ref, sems, xsems, osem):
    n_x = S // (NSUBS[0] * SUB)

    def x_copy(t):
        ts = NSUBS[0] * SUB
        rows = pl.ds(pl.multiple_of(t * ts, ts), ts)
        return pltpu.make_async_copy(x_hbm.at[0, rows], xio_ref.at[rows], xsems.at[t])

    wphi_copy = pltpu.make_async_copy(wphi_hbm, wphi_ref, sems.at[0])
    qkv_copies = [
        pltpu.make_async_copy(wqkv_hbm.at[:, pl.ds(p * D, D)],
                              wqkv_ref.at[:, pl.ds(p * D, D)], sems.at[1 + p])
        for p in range(3)]
    late_copies = [
        pltpu.make_async_copy(src, dst, sems.at[4 + i])
        for i, (src, dst) in enumerate([
            (wo_hbm, wo_ref), (w1t_hbm, w1t_ref), (w2_hbm, w2_ref)])]
    wphi_copy.start()
    for c in qkv_copies:
        c.start()

    def out_copy(t):
        ts = NSUBS[2] * SUB
        rows = pl.ds(pl.multiple_of(t * ts, ts), ts)
        return pltpu.make_async_copy(xio_ref.at[rows], o_hbm.at[0, rows], osem)

    def prep():
        wphi_copy.wait()
        tmpw_ref[...] = jnp.zeros(tmpw_ref.shape, tmpw_ref.dtype)
        for h in range(H):
            tmpw_ref[pl.ds(DH * h, DH), pl.ds(0, DH)] = (
                wphi_ref[h].astype(jnp.float32))
        wphi2 = tmpw_ref[...].astype(jnp.bfloat16)
        RB = 160
        los = [min(128 * b, D - 256) for b in range(D // RB)]
        mts = []
        for b in range(D // RB):
            r = RB * b + lax.broadcasted_iota(jnp.int32, (RB, 128), 0)
            k = lax.broadcasted_iota(jnp.int32, (RB, 128), 1)
            onehot = (k == (r % GROWS) // HG).astype(jnp.bfloat16)
            mfull = _dot_nt(onehot, wphi2[los[b]:los[b] + 256])
            r = RB * b + lax.broadcasted_iota(jnp.int32, (RB, 256), 0)
            c = los[b] + lax.broadcasted_iota(jnp.int32, (RB, 256), 1)
            head_r = (r // GROWS) * HG + r % HG
            mts.append(jnp.where(c // DH == head_r, mfull, 0.0).astype(jnp.bfloat16))
        for part in range(2):
            qkv_copies[part].wait()
            if part == 0:
                x_copy(0).start()
            for b in range(D // RB):
                wat_ref[pl.ds(part * D + RB * b, RB), :] = _dot_nt(
                    mts[b], wqkv_ref[:, pl.ds(part * D + los[b], 256)]).astype(jnp.bfloat16)
        qkv_copies[2].wait()
        for t in range(1, n_x):
            x_copy(t).start()
        for c in late_copies:
            c.start()
        r = lax.broadcasted_iota(jnp.int32, (128, 128), 0)
        c = lax.broadcasted_iota(jnp.int32, (128, 128), 1)
        eye = (r == c).astype(jnp.bfloat16)
        for b in range(D // 128):
            wat_ref[pl.ds(2 * D + 128 * b, 128), :] = _dot_nt(
                eye, wqkv_ref[:, pl.ds(2 * D + 128 * b, 128)]).astype(jnp.bfloat16)
        acc_ref[...] = jnp.zeros(acc_ref.shape, acc_ref.dtype)

    def finalize():
        r = lax.broadcasted_iota(jnp.int32, (VROWS, GPHI), 0)
        c = lax.broadcasted_iota(jnp.int32, (VROWS, GPHI), 1)
        head_r = jnp.where(r < GROWS, r // DH,
                           jnp.where(r < 48, 0, jnp.where(r < 56, 1, (r - 56) // 4)))
        keep = head_r == c % HG
        for g in range(NG):
            kvz_ref[g] = jnp.where(keep, acc_ref[g, :, pl.ds(0, GPHI)], 0.0).astype(jnp.bfloat16)
        acc_ref[...] = jnp.zeros(acc_ref.shape, acc_ref.dtype)

    def sub_cols(t, nsub):
        return [pl.multiple_of((t * nsub + u) * SUB, SUB) for u in range(nsub)]

    def back(cols):
        o_l = []
        for u in range(len(cols)):
            o_parts = []
            for g in range(NG):
                pg = phiq_ref[pl.ds(GPHI * g, GPHI), pl.ds(cols[u], SUB)]
                res = _dot(kvz_ref[g], pg)
                ra = pl.reciprocal(res[40:48] + DEN_EPS, approx=False)
                rb = pl.reciprocal(res[48:56] + DEN_EPS, approx=False)
                rm = pl.reciprocal(res[56:64] + DEN_EPS, approx=False)
                o_parts += [res[0:8] * ra, res[8:16] * ra, res[16:24] * rm,
                            res[24:32] * rb, res[32:40] * rb]
            o_t = jnp.concatenate(o_parts, axis=0)
            o_l.append(o_t.T.astype(jnp.bfloat16))
        x1_l = [xres_ref[pl.ds(cols[u], SUB), :] + _dot(o_l[u], wo_ref[...])
                for u in range(len(cols))]
        h_l = []
        for u in range(len(cols)):
            xn = _layernorm(x1_l[u]).astype(jnp.bfloat16)
            hdn = _dot_nt(xn, w1t_ref[...])
            h_l.append((hdn * jax.nn.sigmoid(hdn)).astype(jnp.bfloat16))
        return [x1_l[u] + _dot(h_l[u], w2_ref[...]) for u in range(len(cols))]

    def front(cols, x_l):
        y_l = []
        for u in range(len(cols)):
            xn = _layernorm(x_l[u]).astype(jnp.bfloat16)
            y_l.append(_dot_nt(wat_ref[...], xn))
        ones = jnp.ones((VROWS - GROWS, SUB), jnp.float32)
        for u in range(len(cols)):
            y_t = y_l[u]
            phiq_ref[:, pl.ds(cols[u], SUB)] = _phi_t(y_t[:D])
            phik = jnp.concatenate(
                [_phi_t(y_t[D:2 * D]), jnp.zeros((128 - GPHI, SUB), jnp.bfloat16)], axis=0)
            v_t = y_t[2 * D:]
            for g in range(NG):
                vaug = jnp.concatenate([v_t[GROWS * g:GROWS * (g + 1)], ones],
                                       axis=0).astype(jnp.bfloat16)
                acc_ref[g] += _dot_nt(vaug, phik[GPHI * g:GPHI * g + 128])

    def phase0(t, carry):
        x_copy(t).wait()
        cols = sub_cols(t, NSUBS[0])
        x_l = [xio_ref[pl.ds(cols[u], SUB), :].astype(jnp.float32) for u in range(len(cols))]
        for u in range(len(cols)):
            xres_ref[pl.ds(cols[u], SUB), :] = x_l[u]
        front(cols, x_l)
        return carry

    def phase1(t, carry):
        cols = sub_cols(t, NSUBS[1])
        x_l = back(cols)
        for u in range(len(cols)):
            xres_ref[pl.ds(cols[u], SUB), :] = x_l[u]
        front(cols, x_l)
        return carry

    def phase2(t, carry):
        cols = sub_cols(t, NSUBS[2])
        x_l = back(cols)
        for u in range(len(cols)):
            xio_ref[pl.ds(cols[u], SUB), :] = x_l[u].astype(xio_ref.dtype)
        out_copy(t).start()
        return carry

    prep()
    lax.fori_loop(0, S // (NSUBS[0] * SUB), phase0, 0)
    finalize()
    for c in late_copies:
        c.wait()
    lax.fori_loop(0, S // (NSUBS[1] * SUB), phase1, 0)
    finalize()
    lax.fori_loop(0, S // (NSUBS[2] * SUB), phase2, 0)

    def drain(t, carry):
        out_copy(t).wait()
        return carry

    lax.fori_loop(0, S // (NSUBS[2] * SUB), drain, 0)


@jax.jit
def pallas_interleave_layers__linear_kernel_hedgehog__dense_activation_silu__prompt_kernel(
    A_x: jax.Array,
    A_wqkv: jax.Array,
    A_w_phi: jax.Array,
    A_wo: jax.Array,
    B_x: jax.Array,
    B_w1: jax.Array,
    B_w2: jax.Array,
):
    del B_x
    hbm = pl.BlockSpec(memory_space=pl.ANY)
    return pl.pallas_call(
        _kernel,
        in_specs=[hbm, hbm, hbm, hbm, hbm, hbm],
        out_specs=hbm,
        out_shape=jax.ShapeDtypeStruct((1, S, D), jnp.bfloat16),
        scratch_shapes=[
            pltpu.VMEM((S, D), jnp.bfloat16),
            pltpu.VMEM((S, D), jnp.float32),
            pltpu.VMEM((2 * D, S), jnp.bfloat16),
            pltpu.VMEM((3 * D, D), jnp.bfloat16),
            pltpu.VMEM((D, 128), jnp.float32),
            pltpu.VMEM((NG, VROWS, 128), jnp.float32),
            pltpu.VMEM((NG, VROWS, GPHI), jnp.bfloat16),
            pltpu.VMEM((D, 3 * D), jnp.bfloat16),
            pltpu.VMEM((H, DH, DH), jnp.bfloat16),
            pltpu.VMEM((D, D), jnp.bfloat16),
            pltpu.VMEM((F, D), jnp.bfloat16),
            pltpu.VMEM((F, D), jnp.bfloat16),
            pltpu.SemaphoreType.DMA((7,)),
            pltpu.SemaphoreType.DMA((S // (NSUBS[0] * SUB),)),
            pltpu.SemaphoreType.DMA(()),
        ],
        compiler_params=pltpu.CompilerParams(
            vmem_limit_bytes=100 * 1024 * 1024,
        ),
    )(A_x, A_wqkv, A_w_phi, A_wo, B_w1.T, B_w2)
```

```python
import jax
import jax.numpy as jnp
from jax import lax
import jax.experimental.pallas as pl
import jax.experimental.pallas.tpu as pltpu

S = 2048
D = 640
H = 32
DH = 20
F = 1728
FM = F // 128 * 128
HG = 2
NG = H // HG
GROWS = HG * DH
GPHI = 2 * GROWS
VROWS = 64

SUB = 128
NSUBS = (8, 2, 4)

LN_EPS = 1e-5
DEN_EPS = 1e-6

_NT_DIMS = (((1,), (1,)), ((), ()))


def _dot(a, b):
    return jnp.dot(a, b, preferred_element_type=jnp.float32)


def _dot_nt(a, b):
    return lax.dot_general(a, b, _NT_DIMS, preferred_element_type=jnp.float32)


def _layernorm(x):
    m = jnp.mean(x, axis=-1, keepdims=True)
    xc = x - m
    v = jnp.mean(xc * xc, axis=-1, keepdims=True)
    return xc * lax.rsqrt(v + LN_EPS)


def _phi_t(p_t):
    ts = p_t.shape[1]
    p = p_t.reshape(NG, 5, 8, ts)

    def allred(x, op):
        x = op(x, pltpu.roll(x, 2, 1))
        x = op(x, pltpu.roll(x, 4, 1))
        return x[:, None]

    pmax = allred(jnp.max(p, axis=1), jnp.maximum)
    pmin = allred(jnp.min(p, axis=1), jnp.minimum)
    ep = jnp.exp(p - pmax)
    en = jnp.exp(pmin - p)
    rp = pl.reciprocal(allred(jnp.sum(ep, axis=1), jnp.add), approx=False)
    rn = pl.reciprocal(allred(jnp.sum(en, axis=1), jnp.add), approx=False)
    phi = jnp.concatenate([ep * rp, en * rn], axis=1)
    return phi.reshape(2 * D, ts).astype(jnp.bfloat16)


def _kernel(x_hbm, wqkv_hbm, wphi_hbm, wo_hbm, w1t_hbm, w2_hbm, o_hbm,
            xio_ref, xres_ref, phiq_ref, wat_ref, tmpw_ref, acc_ref, kvz_ref,
            wqkv_ref, wphi_ref, wo_ref, w1t_ref, w2_ref, sems, xsems, osem):
    n_x = S // (NSUBS[0] * SUB)

    def x_copy(t):
        ts = NSUBS[0] * SUB
        rows = pl.ds(pl.multiple_of(t * ts, ts), ts)
        return pltpu.make_async_copy(x_hbm.at[0, rows], xio_ref.at[rows], xsems.at[t])

    wphi_copy = pltpu.make_async_copy(wphi_hbm, wphi_ref, sems.at[0])
    qkv_copies = [
        pltpu.make_async_copy(wqkv_hbm.at[:, pl.ds(p * D, D)],
                              wqkv_ref.at[:, pl.ds(p * D, D)], sems.at[1 + p])
        for p in range(3)]
    late_copies = [
        pltpu.make_async_copy(src, dst, sems.at[4 + i])
        for i, (src, dst) in enumerate([
            (wo_hbm, wo_ref), (w1t_hbm, w1t_ref), (w2_hbm, w2_ref)])]
    wphi_copy.start()
    for c in qkv_copies:
        c.start()

    def out_copy(col):
        rows = pl.ds(col, SUB)
        return pltpu.make_async_copy(xio_ref.at[rows], o_hbm.at[0, rows], osem)

    def prep():
        wphi_copy.wait()
        tmpw_ref[...] = jnp.zeros(tmpw_ref.shape, tmpw_ref.dtype)
        for h in range(H):
            tmpw_ref[pl.ds(DH * h, DH), pl.ds(0, DH)] = (
                wphi_ref[h].astype(jnp.float32))
        wphi2 = tmpw_ref[...].astype(jnp.bfloat16)
        RB = 160
        los = [min(128 * b, D - 256) for b in range(D // RB)]
        mts = []
        for b in range(D // RB):
            r = RB * b + lax.broadcasted_iota(jnp.int32, (RB, 128), 0)
            k = lax.broadcasted_iota(jnp.int32, (RB, 128), 1)
            onehot = (k == (r % GROWS) // HG).astype(jnp.bfloat16)
            mfull = _dot_nt(onehot, wphi2[los[b]:los[b] + 256])
            r = RB * b + lax.broadcasted_iota(jnp.int32, (RB, 256), 0)
            c = los[b] + lax.broadcasted_iota(jnp.int32, (RB, 256), 1)
            head_r = (r // GROWS) * HG + r % HG
            mts.append(jnp.where(c // DH == head_r, mfull, 0.0).astype(jnp.bfloat16))
        for part in range(2):
            qkv_copies[part].wait()
            if part == 0:
                x_copy(0).start()
            for b in range(D // RB):
                wat_ref[pl.ds(part * D + RB * b, RB), :] = _dot_nt(
                    mts[b], wqkv_ref[:, pl.ds(part * D + los[b], 256)]).astype(jnp.bfloat16)
        qkv_copies[2].wait()
        for t in range(1, n_x):
            x_copy(t).start()
        for c in late_copies:
            c.start()
        r = lax.broadcasted_iota(jnp.int32, (128, 128), 0)
        c = lax.broadcasted_iota(jnp.int32, (128, 128), 1)
        eye = (r == c).astype(jnp.bfloat16)
        for b in range(D // 128):
            wat_ref[pl.ds(2 * D + 128 * b, 128), :] = _dot_nt(
                eye, wqkv_ref[:, pl.ds(2 * D + 128 * b, 128)]).astype(jnp.bfloat16)
        acc_ref[...] = jnp.zeros(acc_ref.shape, acc_ref.dtype)

    def finalize():
        r = lax.broadcasted_iota(jnp.int32, (VROWS, GPHI), 0)
        c = lax.broadcasted_iota(jnp.int32, (VROWS, GPHI), 1)
        head_r = jnp.where(r < GROWS, r // DH,
                           jnp.where(r < 48, 0, jnp.where(r < 56, 1, (r - 56) // 4)))
        keep = head_r == c % HG
        for g in range(NG):
            kvz_ref[g] = jnp.where(keep, acc_ref[g, :, pl.ds(0, GPHI)], 0.0).astype(jnp.bfloat16)
        acc_ref[...] = jnp.zeros(acc_ref.shape, acc_ref.dtype)

    def sub_cols(t, nsub):
        return [pl.multiple_of((t * nsub + u) * SUB, SUB) for u in range(nsub)]

    def back(cols):
        o_l = []
        for u in range(len(cols)):
            o_parts = []
            for g in range(NG):
                pg = phiq_ref[pl.ds(GPHI * g, GPHI), pl.ds(cols[u], SUB)]
                res = _dot(kvz_ref[g], pg)
                ra = pl.reciprocal(res[40:48] + DEN_EPS, approx=False)
                rb = pl.reciprocal(res[48:56] + DEN_EPS, approx=False)
                rm = pl.reciprocal(res[56:64] + DEN_EPS, approx=False)
                o_parts += [res[0:8] * ra, res[8:16] * ra, res[16:24] * rm,
                            res[24:32] * rb, res[32:40] * rb]
            o_t = jnp.concatenate(o_parts, axis=0)
            o_l.append(o_t.T.astype(jnp.bfloat16))
        x1_l = [xres_ref[pl.ds(cols[u], SUB), :] + _dot(o_l[u], wo_ref[...])
                for u in range(len(cols))]
        h_l = []
        for u in range(len(cols)):
            xn = _layernorm(x1_l[u]).astype(jnp.bfloat16)
            h_tail = _dot_nt(w1t_ref[pl.ds(FM, F - FM), :], xn).T
            hdn = jnp.concatenate([_dot_nt(xn, w1t_ref[pl.ds(0, FM), :]), h_tail], axis=1)
            h_l.append((hdn * jax.nn.sigmoid(hdn)).astype(jnp.bfloat16))
        return [x1_l[u] + _dot(h_l[u], w2_ref[...]) for u in range(len(cols))]

    def front(cols, x_l):
        y_l = []
        for u in range(len(cols)):
            xn = _layernorm(x_l[u]).astype(jnp.bfloat16)
            y_l.append(_dot_nt(wat_ref[...], xn))
        ones = jnp.ones((VROWS - GROWS, SUB), jnp.float32)
        for u in range(len(cols)):
            y_t = y_l[u]
            phiq_ref[:, pl.ds(cols[u], SUB)] = _phi_t(y_t[:D])
            phik = jnp.concatenate(
                [_phi_t(y_t[D:2 * D]), jnp.zeros((128 - GPHI, SUB), jnp.bfloat16)], axis=0)
            v_t = y_t[2 * D:]
            for g in range(NG):
                vaug = jnp.concatenate([v_t[GROWS * g:GROWS * (g + 1)], ones],
                                       axis=0).astype(jnp.bfloat16)
                acc_ref[g] += _dot_nt(vaug, phik[GPHI * g:GPHI * g + 128])

    def phase0(t, carry):
        x_copy(t).wait()
        cols = sub_cols(t, NSUBS[0])
        x_l = [xio_ref[pl.ds(cols[u], SUB), :].astype(jnp.float32) for u in range(len(cols))]
        for u in range(len(cols)):
            xres_ref[pl.ds(cols[u], SUB), :] = x_l[u]
        front(cols, x_l)
        return carry

    def phase1(t, carry):
        cols = sub_cols(t, NSUBS[1])
        x_l = back(cols)
        for u in range(len(cols)):
            xres_ref[pl.ds(cols[u], SUB), :] = x_l[u]
        front(cols, x_l)
        return carry

    def phase2(t, carry):
        cols = sub_cols(t, NSUBS[2])
        x_l = back(cols)
        for u in range(len(cols)):
            xio_ref[pl.ds(cols[u], SUB), :] = x_l[u].astype(xio_ref.dtype)
            out_copy(cols[u]).start()
        return carry

    prep()
    lax.fori_loop(0, S // (NSUBS[0] * SUB), phase0, 0)
    finalize()
    for c in late_copies:
        c.wait()
    lax.fori_loop(0, S // (NSUBS[1] * SUB), phase1, 0)
    finalize()
    lax.fori_loop(0, S // (NSUBS[2] * SUB), phase2, 0)

    def drain(k, carry):
        out_copy(pl.multiple_of(k * SUB, SUB)).wait()
        return carry

    lax.fori_loop(0, S // SUB, drain, 0)


@jax.jit
def pallas_interleave_layers__linear_kernel_hedgehog__dense_activation_silu__prompt_kernel(
    A_x: jax.Array,
    A_wqkv: jax.Array,
    A_w_phi: jax.Array,
    A_wo: jax.Array,
    B_x: jax.Array,
    B_w1: jax.Array,
    B_w2: jax.Array,
):
    del B_x
    hbm = pl.BlockSpec(memory_space=pl.ANY)
    return pl.pallas_call(
        _kernel,
        in_specs=[hbm, hbm, hbm, hbm, hbm, hbm],
        out_specs=hbm,
        out_shape=jax.ShapeDtypeStruct((1, S, D), jnp.bfloat16),
        scratch_shapes=[
            pltpu.VMEM((S, D), jnp.bfloat16),
            pltpu.VMEM((S, D), jnp.float32),
            pltpu.VMEM((2 * D, S), jnp.bfloat16),
            pltpu.VMEM((3 * D, D), jnp.bfloat16),
            pltpu.VMEM((D, 128), jnp.float32),
            pltpu.VMEM((NG, VROWS, 128), jnp.float32),
            pltpu.VMEM((NG, VROWS, GPHI), jnp.bfloat16),
            pltpu.VMEM((D, 3 * D), jnp.bfloat16),
            pltpu.VMEM((H, DH, DH), jnp.bfloat16),
            pltpu.VMEM((D, D), jnp.bfloat16),
            pltpu.VMEM((F, D), jnp.bfloat16),
            pltpu.VMEM((F, D), jnp.bfloat16),
            pltpu.SemaphoreType.DMA((7,)),
            pltpu.SemaphoreType.DMA((S // (NSUBS[0] * SUB),)),
            pltpu.SemaphoreType.DMA(()),
        ],
        compiler_params=pltpu.CompilerParams(
            vmem_limit_bytes=100 * 1024 * 1024,
        ),
    )(A_x, A_wqkv, A_w_phi, A_wo, B_w1.T, B_w2)
```
